```python
import jax
import jax.numpy as jnp

def _softmax(x, axis=-1):
    return jax.nn.softmax(x, axis=axis)
def _gelu(x):
    return jax.nn.gelu(x, approximate=True)
def _silu(x):
    return jax.nn.silu(x)
def _sigmoid(x):
    return jax.nn.sigmoid(x)
def _layernorm(x, axis=-1, eps=1e-5):
    m = jnp.mean(x, axis=axis, keepdims=True)
    v = jnp.var(x, axis=axis, keepdims=True)
    return (x - m) / jnp.sqrt(v + eps)
def _scatter_add(tgt, idx, src, axis=0):
    return tgt.at[idx].add(src)
def _segment_sum(src, seg, n):
    return jax.ops.segment_sum(src, seg, n)
class _Rng:
    def __init__(self, key):
        self._k = key
    def _next(self):
        self._k, sub = jax.random.split(self._k)
        return sub
    def normal(self, shape):
        return jax.random.normal(self._next(), shape, dtype=jnp.bfloat16)
    def randint(self, lo, hi, shape):
        return jax.random.randint(self._next(), shape, lo, hi, dtype=jnp.int32)
    def uniform(self, shape, lo=0.0, hi=1.0):
        return jax.random.uniform(self._next(), shape, jnp.bfloat16, lo, hi)
    def permutation(self, n):
        return jax.random.permutation(self._next(), n)


kernel_name = 'standalone__modern_conv_block_convnext_v2__vision'

def setup_inputs():
    _rng = _Rng(jax.random.key(int.from_bytes(__import__("os").urandom(4), "little")))
    _w = (lambda a: (lambda t: t.astype(jnp.bfloat16) if jnp.issubdtype(t.dtype, jnp.floating) else t)(jnp.asarray(a)))
    H = W = 512
    C = 96
    K = 3
    return {
        "x": _w((lambda *s: _rng.normal(s) * 0.05)(1, H, W, C)),
        "dw": _w((lambda *s: _rng.normal(s) * 0.05)(K, K, C)),
        "w1": _w((lambda *s: _rng.normal(s) * 0.05)(C, 4 * C)),
        "w2": _w((lambda *s: _rng.normal(s) * 0.05)(4 * C, C)),
        "grn_gamma": _w((lambda *s: _rng.normal(s) * 0.05)(4 * C)),
        "grn_beta": _w((lambda *s: _rng.normal(s) * 0.05)(4 * C)),
    }

def reference(x, dw, w1, w2, grn_gamma, grn_beta):
    B, H, W, C = x.shape
    K = dw.shape[0]
    pad = K // 2
    xp = jnp.pad(x, ((0,0),(pad,pad),(pad,pad),(0,0)))
    out = jnp.zeros_like(x)
    for i in range(K):
        for j in range(K):
            out = out + xp[:, i:i+H, j:j+W, :] * dw[i, j][None, None, None, :]
    h = _layernorm(out, axis=-1)
    h = jnp.einsum('bhwc,ce->bhwe', h, w1)
    h = _gelu(h)
    gx = jnp.sqrt((h * h).sum(axis=(1, 2), keepdims=True) + 1e-6)
    nx = gx / (gx.mean(axis=-1, keepdims=True) + 1e-6)
    h = grn_gamma * (h * nx) + grn_beta + h
    h = jnp.einsum('bhwe,ec->bhwc', h, w2)
    return x + h
```

```python
import numpy as np
import jax
import jax.numpy as jnp
from jax import lax
import jax.experimental.pallas as pl
import jax.experimental.pallas.tpu as pltpu

_C1 = float(np.sqrt(2.0 / np.pi))
_C2 = _C1 * 0.044715
_S = _C2 ** (1.0 / 3.0)
_K = _C1 / _S
_GS = 0.5 / _S
f32, bf16, u32 = jnp.float32, jnp.bfloat16, jnp.uint32


def build(x, dw, w1, w2, gamma, beta, U=4, NB=4, split=2, vmem=128 * 2**20, flag=None, pat2='PFA'):
    flags = {flag: True} if flag else None
    _, H, W, C = x.shape
    E = w1.shape[1]
    T = W // 128
    G = C // 8
    P = H // 2
    nb = P // U
    LA = 2
    x5 = jnp.transpose(x.reshape(H, W, C), (0, 2, 1)).reshape(P, 2, G, 8, W)

    def kernel(x_hbm, dw_ref, w1_ref, w2t_ref, g_ref, b_ref, o_hbm,
               buf, pro, xs, ob, rsb, acc, dm, w1t, w2s, bias, ge, yc, hc, sin, sout, spro):
        lane = lax.broadcasted_iota(jnp.int32, (8, 128), 1)
        first = lane == 0
        last = lane == 127
        zero = jnp.zeros((8, 128), u32)

        def cp(src, dst, sem):
            return pltpu.make_async_copy(src, dst, sem)

        def in1(b, n0=U, n1=U):
            s = b % NB
            return (cp(x_hbm.at[pl.ds(b * U + 1, n0), 1], buf.at[s, pl.ds(0, n0), :, pl.ds(0, 8)], sin.at[s, 0]),
                    cp(x_hbm.at[pl.ds(b * U + 2, n1), 0], buf.at[s, pl.ds(0, n1), :, pl.ds(8, 8)], sin.at[s, 1]))

        def in2(b):
            s = (b + nb) % NB
            return tuple(cp(x_hbm.at[pl.ds(b * U, U), j], buf.at[s, :, :, pl.ds(8 * j, 8)], sin.at[s, j]) for j in range(2))

        def out2(b):
            s = (b + nb) % NB
            return tuple(cp(buf.at[s, :, :, pl.ds(8 * j, 8)], o_hbm.at[pl.ds(b * U, U), j], sout.at[s, j]) for j in range(2))

        def start(cs):
            for c in cs:
                c.start()

        def wait(cs):
            for c in cs:
                c.wait()

        pro_cp = (cp(x_hbm.at[pl.ds(0, 1), 1], pro.at[pl.ds(1, 1), :, pl.ds(0, 8)], spro.at[0]),
                  cp(x_hbm.at[pl.ds(0, 2), 0], pro.at[:, :, pl.ds(8, 8)], spro.at[1]))
        start(pro_cp)
        for b in range(LA):
            start(in1(b))

        w = w1_ref[...].astype(f32)
        w = w - jnp.sum(w, axis=0, keepdims=True) * (1.0 / C)
        w = jnp.concatenate([w, jnp.zeros((128 - C, E), f32)], axis=0)
        w1t[...] = pltpu.bitcast(w.T.astype(bf16), u32)
        d = jnp.concatenate([dw_ref[...].astype(f32), jnp.zeros((9, 128 - C), f32)], axis=1)
        dt = jnp.concatenate([d, jnp.zeros((128 - 9, 128), f32)], axis=0).T
        sub = lax.broadcasted_iota(jnp.int32, (8, 128), 0)
        for g in range(G):
            cols = [jnp.broadcast_to(dt[8 * g:8 * g + 8, t:t + 1], (8, 128)) for t in range(9)]
            halves = []
            for j in range(2):
                m = jnp.zeros((8, 128), f32)
                for r in range(4):
                    if 0 <= r - j < 3:
                        for s in range(3):
                            base = (r // 2) * 48 + s * 16 + (r % 2) * 8
                            m = jnp.where(lane == base + sub, cols[(r - j) * 3 + s], m)
                halves.append(m)
            dm[g] = pltpu.bitcast(jnp.concatenate(halves, axis=0).astype(bf16), u32)
        acc[...] = jnp.zeros_like(acc)
        pro[0, :, 0:8, :] = jnp.zeros((G, 8, W), bf16)

        def shifts(v):
            tl = [v[:, 128 * t:128 * t + 128] for t in range(T)]
            a = [pltpu.roll(q, 1, 1) for q in tl]
            b = [pltpu.roll(q, 127, 1) for q in tl]
            l = [jnp.where(first, a[t - 1] if t > 0 else zero, a[t]) for t in range(T)]
            r = [jnp.where(last, b[t + 1] if t < T - 1 else zero, b[t]) for t in range(T)]
            return jnp.concatenate([jnp.concatenate(l, axis=1), v, jnp.concatenate(r, axis=1)], axis=0)

        class Conv:
            def __init__(self, src):
                self.src = src
                self.o = []

            def group(self):
                g = len(self.o)
                old = xs[g]
                new = shifts(pltpu.bitcast(self.src(g), u32))
                xs[g] = new
                rhs = pltpu.bitcast(jnp.concatenate([old, new], axis=0), bf16)
                lhs = pltpu.bitcast(dm[g], bf16)[:, :96]
                o = jnp.dot(lhs, rhs, preferred_element_type=f32)
                self.o.append(o)
                self.s1 = o if g == 0 else self.s1 + o
                self.s2 = o * o if g == 0 else self.s2 + o * o

            def done(self):
                for g in range(G):
                    for j in range(2):
                        ob[j, 8 * g:8 * g + 8, :] = self.o[g][8 * j:8 * j + 8]
                for j in range(2):
                    m = jnp.sum(self.s1[8 * j:8 * j + 8], axis=0, keepdims=True) * (1.0 / C)
                    q = jnp.sum(self.s2[8 * j:8 * j + 8], axis=0, keepdims=True) * (1.0 / C)
                    v = jnp.maximum(q - m * m, 0.0)
                    rsb[j] = jnp.broadcast_to(lax.rsqrt(v + 1e-5) * _S, (8, W))

        def gelu(z):
            return z * (1.0 + jnp.tanh(z * (_K + z * z)))

        def step1(s, u, k):
            yf = [ob[j] * jnp.concatenate([rsb[j]] * G, axis=0) for j in range(2)]
            yc[k] = yf[0].astype(bf16)
            ys = [yc[k], yf[1].astype(bf16)]
            cv = Conv(lambda g: buf[s, u, g])
            n = E // split
            slots = [(j, c) for j in (1, 0) for c in range(split)]
            for i, (j, c) in enumerate(slots):
                wl = pltpu.bitcast(w1t[n // 2 * c:n // 2 * (c + 1), :], bf16)[:, :C]
                g = gelu(jnp.dot(wl, ys[j], preferred_element_type=f32))
                g2 = g * g
                sq = g2[:, 0:128]
                for t in range(1, T):
                    sq = sq + g2[:, 128 * t:128 * t + 128]
                acc[n * c:n * c + n, :] += sq
                if j == 1:
                    hc[k, n * c:n * c + n, :] = g.astype(bf16)
                while len(cv.o) < min(G, G * (i + 1) / (len(slots) - 1)):
                    cv.group()
            cv.done()

        wait(pro_cp)
        for g in range(G):
            xs[g] = shifts(pltpu.bitcast(pro[0, g], u32))
        cv = Conv(lambda g: pro[1, g])
        for g in range(G):
            cv.group()
        cv.done()

        def body1(b, _):
            s = b % NB

            @pl.when(b + LA < nb - 1)
            def _():
                start(in1(b + LA))

            @pl.when(b + LA == nb - 1)
            def _():
                start(in1(nb - 1, U - 1, U - 2))

            @pl.when(b + LA >= nb)
            def _():
                start(in2(b + LA - nb))

            @pl.when(b < nb - 1)
            def _():
                wait(in1(b))

            @pl.when(b == nb - 1)
            def _():
                wait(in1(nb - 1, U - 1, U - 2))
                buf[(nb - 1) % NB, U - 2, :, 8:16, :] = jnp.zeros((G, 8, W), bf16)

            for u in range(U):
                step1(s, u, b * U + u)
            return 0

        lax.fori_loop(0, nb, body1, 0)

        ss = jnp.sum(acc[...].T, axis=0, keepdims=True) * (_GS * _GS)
        gx = jnp.sqrt(ss + 1e-6)
        nx = gx / (jnp.mean(gx, axis=-1, keepdims=True) + 1e-6)
        sc = (g_ref[...].astype(f32) * nx + 1.0) * _GS
        w = w2t_ref[...].astype(f32)
        w2s[...] = pltpu.bitcast((w * sc).astype(bf16), u32)
        bb = jnp.sum(w * b_ref[...].astype(f32), axis=-1, keepdims=True)
        bias[...] = jnp.broadcast_to(bb, bias.shape)

        def produce(k, slot):
            wl = pltpu.bitcast(w1t[...], bf16)[:, :C]
            ge[slot] = gelu(jnp.dot(wl, yc[k], preferred_element_type=f32)).astype(bf16)

        def finish(s, u, j, gb):
            o = jnp.dot(pltpu.bitcast(w2s[...], bf16), gb, preferred_element_type=f32)
            o = o + jnp.concatenate([bias[...]] * T, axis=1)
            for g in range(G):
                r = buf[s, u, g, 8 * j:8 * j + 8, :].astype(f32) + o[8 * g:8 * g + 8]
                buf[s, u, g, 8 * j:8 * j + 8, :] = r.astype(bf16)

        produce(0, 0)

        def body2(b, _):
            s = (b + nb) % NB

            @pl.when(b >= NB - LA)
            def _():
                wait(out2(b - (NB - LA)))

            @pl.when(b + LA < nb)
            def _():
                start(in2(b + LA))

            wait(in2(b))
            for u in range(U):
                k = b * U + u
                for ch in pat2:
                    if ch == 'P':
                        produce(jnp.minimum(k + 1, P - 1), (u + 1) % 2)
                    elif ch == 'F':
                        finish(s, u, 0, ge[u % 2])
                    else:
                        finish(s, u, 1, hc[k])
            start(out2(b))
            return 0

        lax.fori_loop(0, nb, body2, 0)
        for b in range(nb - (NB - LA), nb):
            wait(out2(b))

    vm = pl.BlockSpec(memory_space=pltpu.VMEM)
    out = pl.pallas_call(
        kernel,
        in_specs=[pl.BlockSpec(memory_space=pl.ANY), vm, vm, vm, vm, vm],
        out_specs=pl.BlockSpec(memory_space=pl.ANY),
        out_shape=jax.ShapeDtypeStruct(x5.shape, x.dtype),
        scratch_shapes=[
            pltpu.VMEM((NB, U, G, 16, W), bf16),
            pltpu.VMEM((2, G, 16, W), bf16),
            pltpu.VMEM((G, 24, W), u32),
            pltpu.VMEM((2, C, W), f32),
            pltpu.VMEM((2, 8, W), f32),
            pltpu.VMEM((E, 128), f32),
            pltpu.VMEM((G, 8, 128), u32),
            pltpu.VMEM((E // 2, 128), u32),
            pltpu.VMEM((C // 2, E), u32),
            pltpu.VMEM((C, 128), f32),
            pltpu.VMEM((2, E, W), bf16),
            pltpu.VMEM((P, C, W), bf16),
            pltpu.VMEM((P, E, W), bf16),
            pltpu.SemaphoreType.DMA((NB, 2)),
            pltpu.SemaphoreType.DMA((NB, 2)),
            pltpu.SemaphoreType.DMA((2,)),
        ],
        compiler_params=pltpu.CompilerParams(vmem_limit_bytes=vmem, flags=flags),
    )(x5, dw.reshape(9, C), w1, w2.T, gamma.reshape(1, E), beta.reshape(1, E))
    return jnp.transpose(out.reshape(H, C, W), (0, 2, 1)).reshape(x.shape)


@jax.jit
def pallas_standalone__modern_conv_block_convnext_v2__vision_kernel(x, dw, w1, w2, grn_gamma, grn_beta):
    return build(x, dw, w1, w2, grn_gamma, grn_beta)
```

```python
import numpy as np
import jax
import jax.numpy as jnp
from jax import lax
import jax.experimental.pallas as pl
import jax.experimental.pallas.tpu as pltpu

_C1 = float(np.sqrt(2.0 / np.pi))
_C2 = _C1 * 0.044715
_S = _C2 ** (1.0 / 3.0)
_K = _C1 / _S
_GS = 0.5 / _S
f32, bf16, u32 = jnp.float32, jnp.bfloat16, jnp.uint32


def build(x, dw, w1, w2, gamma, beta, U=8, sched='8C4M8C4M8C4M8M8M8', vmem=128 * 2**20, flag=None, order=(1, 0), late=True, static=False):
    flags = {flag: True} if flag else None
    _, H, W, C = x.shape
    E = w1.shape[1]
    T = W // 128
    G = C // 8
    P = H // 2
    nb = P // U
    x5 = jnp.transpose(x.reshape(H, W, C), (0, 2, 1)).reshape(P, 2, G, 8, W)
    import re
    toks = [(a or 'M', int(n)) for a, n in re.findall(r'([MC]?)(\d+)', sched)]

    def kernel(x_hbm, dw_ref, w1_ref, w2t_ref, g_ref, b_ref, o_hbm,
               buf, w1t, w2s, bias, yc, hc, sin, sout):
        xu = x_hbm.bitcast(u32)
        ou = o_hbm.bitcast(u32)
        lane = lax.broadcasted_iota(jnp.int32, (8, 128), 1)
        sub = lax.broadcasted_iota(jnp.int32, (8, 128), 0)
        first = lane == 0
        last = lane == 127
        zero = jnp.zeros((8, 128), u32)

        def cp(src, dst, sem):
            return pltpu.make_async_copy(src, dst, sem)

        def in1(b):
            s = (b + 1) % 2
            cs = []
            for j in range(2):
                want = b * U + 1 + j
                got = jnp.minimum(want, P - U)
                cs.append(cp(xu.at[pl.ds(got, U), 1 - j],
                             buf.at[pl.ds(2 + s * U - (want - got), U), :, pl.ds(4 * j, 4)], sin.at[s, j]))
            return cs

        def in2(b, s, sem=sin):
            return [cp(xu.at[pl.ds(b * U, U), j], buf.at[pl.ds(2 + s * U, U), :, pl.ds(4 * j, 4)], sem.at[s, j]) for j in range(2)]

        def out2(b, s):
            return [cp(buf.at[pl.ds(2 + s * U, U), :, pl.ds(4 * j, 4)], ou.at[pl.ds(b * U, U), j], sout.at[s, j]) for j in range(2)]

        def start(cs):
            for c in cs:
                c.start()

        def wait(cs):
            for c in cs:
                c.wait()

        def gelu(z):
            return z * (1.0 + jnp.tanh(z * (_K + z * z)))

        def pass1(xs, ob, rsb, stt, acc, dm):
            pro = (cp(xu.at[pl.ds(0, 1), 1], buf.at[pl.ds(1, 1), :, pl.ds(0, 4)], sin.at[0, 0]),
                   cp(xu.at[pl.ds(0, 2), 0], buf.at[pl.ds(0, 2), :, pl.ds(4, 4)], sin.at[0, 1]))
            start(pro)
            start(in1(0))
            buf[0, :, 0:4, :] = jnp.zeros((G, 4, W), u32)

            w = w1_ref[...].astype(f32)
            w = w - jnp.sum(w, axis=0, keepdims=True) * (1.0 / C)
            w = jnp.concatenate([w, jnp.zeros((128 - C, E), f32)], axis=0)
            w1t[...] = pltpu.bitcast(w.T.astype(bf16), u32)
            d = jnp.concatenate([dw_ref[i].astype(f32) for i in range(3)], axis=0)
            d = jnp.concatenate([d, jnp.zeros((9, 128 - C), f32)], axis=1)
            dt = jnp.concatenate([d, jnp.zeros((128 - 9, 128), f32)], axis=0).T
            pad_row = (lane >= 48) & (lane % 16 >= 8)
            for g in range(G):
                cols = [jnp.broadcast_to(dt[8 * g:8 * g + 8, t:t + 1], (8, 128)) for t in range(9)]
                halves = []
                for j in range(2):
                    m = jnp.zeros((8, 128), f32)
                    for r in range(4):
                        if 0 <= r - j < 3:
                            for s in range(3):
                                base = (r // 2) * 48 + s * 16 + (r % 2) * 8
                                m = jnp.where(lane == base + sub, cols[(r - j) * 3 + s], m)
                    halves.append(m)
                dm[0, g] = pltpu.bitcast(jnp.concatenate(halves, axis=0).astype(bf16), u32)
                halves[1] = jnp.where(pad_row, 0.0, halves[1])
                dm[1, g] = pltpu.bitcast(jnp.concatenate(halves, axis=0).astype(bf16), u32)
            acc[...] = jnp.zeros_like(acc)

            def shifts(v):
                tl = [v[:, 128 * t:128 * t + 128] for t in range(T)]
                a = [pltpu.roll(q, 1, 1) for q in tl]
                b = [pltpu.roll(q, 127, 1) for q in tl]
                l = [jnp.where(first, a[t - 1] if t > 0 else zero, a[t]) for t in range(T)]
                r = [jnp.where(last, b[t + 1] if t < T - 1 else zero, b[t]) for t in range(T)]
                return jnp.concatenate([jnp.concatenate(l, axis=1), v, jnp.concatenate(r, axis=1)], axis=0)

            class Conv:
                def __init__(self, s, sel):
                    self.s, self.sel, self.n, self.o = s, sel, 0, []

                def put(self, g, o):
                    for j in range(2):
                        ob[j, 8 * g:8 * g + 8, :] = o[8 * j:8 * j + 8]

                def group(self):
                    g = self.n
                    self.n += 1
                    old = xs[g]
                    new = shifts(self.s[g])
                    xs[g] = new
                    rhs = pltpu.bitcast(jnp.concatenate([old, new], axis=0), bf16)
                    lhs = pltpu.bitcast(dm[self.sel, g], bf16)[:, :96]
                    o = jnp.dot(lhs, rhs, preferred_element_type=f32)
                    self.o.append(o)
                    if not late:
                        self.put(g, o)
                    self.s1 = o if g == 0 else self.s1 + o
                    self.s2 = o * o if g == 0 else self.s2 + o * o
                    if self.n == G:
                        self.done()

                def done(self):
                    if late:
                        for g in range(G):
                            self.put(g, self.o[g])
                    for q, st in enumerate((self.s1, self.s2)):
                        for j in range(2):
                            for t in range(T):
                                i = j * T + t
                                stt[q, 8 * i:8 * i + 8, :] = st[8 * j:8 * j + 8, 128 * t:128 * t + 128]
                    tot = []
                    for q in range(2):
                        p = [stt[q, pl.ds(i, 8, stride=8), :] for i in range(8)]
                        tot.append((((p[0] + p[1]) + (p[2] + p[3])) + ((p[4] + p[5]) + (p[6] + p[7]))) * (1.0 / C))
                    v = jnp.maximum(tot[1] - tot[0] * tot[0], 0.0)
                    rsb[...] = lax.rsqrt(v + 1e-5) * _S

            def norm(j):
                rs = jnp.concatenate([jnp.broadcast_to(rsb[j * T + t:j * T + t + 1, :], (8, 128)) for t in range(T)], axis=1)
                return (ob[j] * jnp.concatenate([rs] * G, axis=0)).astype(bf16)

            def step1(blk, u, k):
                y1 = norm(1)
                yc[k] = norm(0)
                ys = [yc[k], y1]
                cv = Conv(blk.at[u], (k == P - 2).astype(jnp.int32) if u == (P - 2) % U else 0)
                pos = 0
                for kind, n in toks:
                    if kind == 'C':
                        for _ in range(n):
                            cv.group()
                        continue
                    j = order[pos // (E // 16)]
                    a = 16 * (pos % (E // 16))
                    b = a + 16 * n
                    pos += n
                    wl = pltpu.bitcast(w1t[a // 2:b // 2, :], bf16)[:, :C]
                    g = gelu(jnp.dot(wl, ys[j], preferred_element_type=f32))
                    g2 = g * g
                    sq = g2[:, 0:128]
                    for t in range(1, T):
                        sq = sq + g2[:, 128 * t:128 * t + 128]
                    acc[a:b, :] += sq
                    if j == 1:
                        hc[k, a:b, :] = g.astype(bf16)
                assert cv.n == G and pos == 2 * E // 16

            wait(pro)
            for g in range(G):
                xs[g] = shifts(buf[0, g])
            cv = Conv(buf.at[1], 0)
            for g in range(G):
                cv.group()

            def body1(b, _):
                wait(in1(b))

                @pl.when(b + 1 < nb)
                def _():
                    start(in1(b + 1))

                @pl.when(b + 1 == nb)
                def _():
                    start(in2(0, 1))
                    start(in2(1, 2))

                blk = buf.at[pl.ds(2 + (b + 1) % 2 * U, U)]
                for u in range(U):
                    step1(blk, u, b * U + u)
                return 0

            lax.fori_loop(0, nb, body1, 0)

            ss = jnp.sum(acc[...].T, axis=0, keepdims=True) * (_GS * _GS)
            gx = jnp.sqrt(ss + 1e-6)
            nx = gx / (jnp.mean(gx, axis=-1, keepdims=True) + 1e-6)
            sc = (g_ref[...].astype(f32).reshape(1, E) * nx + 1.0) * _GS
            w = w2t_ref[...].astype(f32)
            w2s[...] = pltpu.bitcast((w * sc).astype(bf16), u32)
            bb = jnp.sum(w * b_ref[...].astype(f32).reshape(1, E), axis=-1, keepdims=True)
            bias[...] = jnp.broadcast_to(bb, bias.shape)

        def pass2(ge):
            def mm2(gb):
                o = jnp.dot(pltpu.bitcast(w2s[...], bf16), gb, preferred_element_type=f32)
                return o + jnp.concatenate([bias[...]] * T, axis=1)

            def body2(b, s):
                sn = jnp.where(s == 2, 0, s + 1)

                @pl.when(b >= 2)
                def _():
                    wait(out2(0, sn))

                @pl.when((b >= 1) & (b + 1 < nb))
                def _():
                    start(in2(b + 1, sn))

                wait(in2(0, s))
                blk = buf.at[pl.ds(2 + s * U, U)]
                for u in range(U):
                    k = b * U + u
                    wl = pltpu.bitcast(w1t[...], bf16)[:, :C]
                    ge[...] = gelu(jnp.dot(wl, yc[k], preferred_element_type=f32)).astype(bf16)
                    o1 = mm2(hc[k])
                    o0 = mm2(ge[...])
                    for g in range(G):
                        o = jnp.concatenate([o0[8 * g:8 * g + 8], o1[8 * g:8 * g + 8]], axis=0)
                        r = pltpu.bitcast(blk[u, g], bf16).astype(f32) + o
                        blk[u, g] = pltpu.bitcast(r.astype(bf16), u32)
                start(out2(b, s))
                return sn

            lax.fori_loop(0, nb, body2, 1)
            for b in range(nb - 2, nb):
                wait(out2(0, (b + 1) % 3))

        pl.run_scoped(pass1,
                      pltpu.VMEM((G, 24, W), u32),
                      pltpu.VMEM((2, C, W), f32),
                      pltpu.VMEM((8, 128), f32),
                      pltpu.VMEM((2, 64, 128), f32),
                      pltpu.VMEM((E, 128), f32),
                      pltpu.VMEM((2, G, 8, 128), u32))
        pl.run_scoped(pass2, pltpu.VMEM((E, W), bf16))

    vm = pl.BlockSpec(memory_space=pltpu.VMEM)
    out = pl.pallas_call(
        kernel,
        in_specs=[pl.BlockSpec(memory_space=pl.ANY), vm, vm, vm, vm, vm],
        out_specs=pl.BlockSpec(memory_space=pl.ANY),
        out_shape=jax.ShapeDtypeStruct(x5.shape, x.dtype),
        scratch_shapes=[
            pltpu.VMEM((2 + 3 * U, G, 8, W), u32),
            pltpu.VMEM((E // 2, 128), u32),
            pltpu.VMEM((C // 2, E), u32),
            pltpu.VMEM((C, 128), f32),
            pltpu.VMEM((P, C, W), bf16),
            pltpu.VMEM((P, E, W), bf16),
            pltpu.SemaphoreType.DMA((3, 2)),
            pltpu.SemaphoreType.DMA((3, 2)),
        ],
        compiler_params=pltpu.CompilerParams(vmem_limit_bytes=vmem, flags=flags),
    )(x5, dw, w1, w2.T, gamma, beta)
    return jnp.transpose(out.reshape(H, C, W), (0, 2, 1)).reshape(x.shape)


@jax.jit
def pallas_standalone__modern_conv_block_convnext_v2__vision_kernel(x, dw, w1, w2, grn_gamma, grn_beta):
    return build(x, dw, w1, w2, grn_gamma, grn_beta)
```

```python
import numpy as np
import jax
import jax.numpy as jnp
from jax import lax
import jax.experimental.pallas as pl
import jax.experimental.pallas.tpu as pltpu

_C1 = float(np.sqrt(2.0 / np.pi))
_C2 = _C1 * 0.044715
_S = _C2 ** (1.0 / 3.0)
_K = _C1 / _S
_GS = 0.5 / _S
f32, bf16, u32 = jnp.float32, jnp.bfloat16, jnp.uint32


def build(x, dw, w1, w2, gamma, beta, sched='8C4M8C4M8C4M12M12', pat='A6A6A6A6A6A7A7A7A7APPF7FPPF7FPPFF', vmem=128 * 2**20, flag=None, order=(1, 0), late=True, SS=9, pri=0, tp=[0, 2], nw=128, ks=384):
    U = 8
    flags = {flag: True} if flag else None
    _, H, W, C = x.shape
    E = w1.shape[1]
    T = W // 128
    G = C // 8
    P = H // 2
    nb = P // U
    R = 2 * U
    NE = 6
    erows = list(range(2, 2 + NE))
    arows = [r for r in range(R) if r not in erows]
    Q = E // C
    S = Q * (R - NE)
    x5 = jnp.transpose(x.reshape(H, W, C), (0, 2, 1)).reshape(P, 2, G, 8, W)
    import re
    toks = [(a or 'M', int(n)) for a, n in re.findall(r'([MC]?)(\d+)', sched)]

    def kernel(x_hbm, dw_ref, w1_ref, w2t_ref, g_ref, b_ref, o_hbm,
               buf, w1t, w2s, dwb, rsc, hc, sin, sout):
        bias = dwb.at[9]
        xu = x_hbm.bitcast(u32)
        lane = lax.broadcasted_iota(jnp.int32, (8, 128), 1)
        sub = lax.broadcasted_iota(jnp.int32, (8, 128), 0)
        first = lane == 0
        last = lane == 127
        zero = jnp.zeros((8, 128), u32)

        def cp(src, dst, sem):
            return pltpu.make_async_copy(src, dst, sem)

        def in1(b):
            s = (b + 1) % 2
            cs = []
            for j in range(2):
                want = b * U + 1 + j
                got = jnp.minimum(want, P - U)
                cs.append(cp(xu.at[pl.ds(got, U), 1 - j],
                             buf.at[pl.ds(2 + s * U - (want - got), U), :, pl.ds(4 * j, 4)], sin.at[s, j]))
            return cs

        def in2(b):
            s = (b + 1) % 2
            return [cp(xu.at[pl.ds(b * U, U), j], buf.at[pl.ds(2 + s * U, U), :, pl.ds(4 * j, 4)], sin.at[s, j]) for j in range(2)]

        def out2(b):
            return [cp(hc.at[pl.ds(1 + b * S, R)], o_hbm.at[pl.ds(b * R, R)], sout.at[b % 4])]

        def start(cs):
            for c in cs:
                c.start()

        def wait(cs):
            for c in cs:
                c.wait()

        def gelu(z):
            return z * (1.0 + jnp.tanh(z * (_K + z * z)))

        def pass1(xs, ob, rsb, stt, acc, dm):
            pro = (cp(xu.at[pl.ds(0, 1), 1], buf.at[pl.ds(1, 1), :, pl.ds(0, 4)], sin.at[0, 0]),
                   cp(xu.at[pl.ds(0, 2), 0], buf.at[pl.ds(0, 2), :, pl.ds(4, 4)], sin.at[0, 1]))
            start(pro)
            start(in1(0))
            buf[0, :, 0:4, :] = jnp.zeros((G, 4, W), u32)

            w = w1_ref[...].astype(f32)
            w = w - jnp.sum(w, axis=0, keepdims=True) * (1.0 / C)
            w = jnp.concatenate([w, jnp.zeros((128 - C, E), f32)], axis=0)
            w1t[...] = pltpu.bitcast(w.T.astype(bf16), u32)
            d = jnp.concatenate([dw_ref[i].astype(f32) for i in range(3)], axis=0)
            d = jnp.concatenate([d, jnp.zeros((9, 128 - C), f32)], axis=1)
            dt = jnp.concatenate([d, jnp.zeros((128 - 9, 128), f32)], axis=0).T
            pad_row = (lane >= 48) & (lane % 16 >= 8)
            for g in range(G):
                cols = [jnp.broadcast_to(dt[8 * g:8 * g + 8, t:t + 1], (8, 128)) for t in range(9)]
                for t in range(9):
                    dwb[t, 8 * g:8 * g + 8, :] = cols[t]
                hc[0, 8 * g:8 * g + 8, 0:128 * len(tp)] = jnp.concatenate([cols[t] for t in tp], axis=1).astype(bf16)
                halves = []
                for j in range(2):
                    m = jnp.zeros((8, 128), f32)
                    for r in range(4):
                        if 0 <= r - j < 3:
                            for s in range(3):
                                base = (r // 2) * 48 + s * 16 + (r % 2) * 8
                                m = jnp.where(lane == base + sub, cols[(r - j) * 3 + s], m)
                    halves.append(m)
                dm[0, g] = pltpu.bitcast(jnp.concatenate(halves, axis=0).astype(bf16), u32)
                halves[1] = jnp.where(pad_row, 0.0, halves[1])
                dm[1, g] = pltpu.bitcast(jnp.concatenate(halves, axis=0).astype(bf16), u32)
            acc[...] = jnp.zeros_like(acc)

            def shifts(v):
                tl = [v[:, 128 * t:128 * t + 128] for t in range(T)]
                a = [pltpu.roll(q, 1, 1) for q in tl]
                b = [pltpu.roll(q, 127, 1) for q in tl]
                l = [jnp.where(first, a[t - 1] if t > 0 else zero, a[t]) for t in range(T)]
                r = [jnp.where(last, b[t + 1] if t < T - 1 else zero, b[t]) for t in range(T)]
                return jnp.concatenate([jnp.concatenate(l, axis=1), v, jnp.concatenate(r, axis=1)], axis=0)

            class Conv:
                def __init__(self, s, sel):
                    self.s, self.sel, self.n, self.o = s, sel, 0, []

                def put(self, g, o):
                    for j in range(2):
                        ob[j, 8 * g:8 * g + 8, :] = o[8 * j:8 * j + 8]

                def group(self):
                    g = self.n
                    self.n += 1
                    old = xs[g]
                    new = shifts(self.s[g])
                    xs[g] = new
                    rhs = pltpu.bitcast(jnp.concatenate([old, new], axis=0), bf16)
                    lhs = pltpu.bitcast(dm[self.sel, g], bf16)[:, :96]
                    o = jnp.dot(lhs, rhs, preferred_element_type=f32)
                    self.o.append(o)
                    if not late:
                        self.put(g, o)
                    self.s1 = o if g == 0 else self.s1 + o
                    self.s2 = o * o if g == 0 else self.s2 + o * o
                    if self.n == G:
                        self.done()

                def done(self):
                    if late:
                        for g in range(G):
                            self.put(g, self.o[g])
                    for q, st in enumerate((self.s1, self.s2)):
                        for j in range(2):
                            for t in range(T):
                                i = j * T + t
                                stt[q, SS * i:SS * i + 8, :] = st[8 * j:8 * j + 8, 128 * t:128 * t + 128]
                    tot = []
                    for q in range(2):
                        p = [stt[q, pl.ds(i, 8, stride=SS), :] for i in range(8)]
                        tot.append((((p[0] + p[1]) + (p[2] + p[3])) + ((p[4] + p[5]) + (p[6] + p[7]))) * (1.0 / C))
                    v = jnp.maximum(tot[1] - tot[0] * tot[0], 0.0)
                    rsb[...] = lax.rsqrt(v + 1e-5) * _S

            def norm(j):
                rs = jnp.concatenate([jnp.broadcast_to(rsb[j * T + t:j * T + t + 1, :], (8, 128)) for t in range(T)], axis=1)
                return (ob[j] * jnp.concatenate([rs] * G, axis=0)).astype(bf16)

            def step1(blk, hb, bi, u):
                ys = [norm(0), norm(1)]
                if 2 * u in erows:
                    rsc[bi, erows.index(2 * u) // 2] = rsb[...]
                cv = Conv(blk.at[u], (bi == nb - 1).astype(jnp.int32) if u == U - 2 else 0)
                pos = 0
                for kind, n in toks:
                    if kind == 'C':
                        for _ in range(n):
                            cv.group()
                        continue
                    j = order[pos // (E // 16)]
                    a = 16 * (pos % (E // 16))
                    b = a + 16 * n
                    pos += n
                    wl = pltpu.bitcast(w1t[a // 2:b // 2, :], bf16)[:, :C]
                    g = gelu(jnp.dot(wl, ys[j], preferred_element_type=f32))
                    g2 = g * g
                    sq = g2[:, 0:128]
                    for t in range(1, T):
                        sq = sq + g2[:, 128 * t:128 * t + 128]
                    acc[a:b, :] += sq
                    if 2 * u + j in arows:
                        q = Q * arows.index(2 * u + j)
                        for c in range(a, b, 16):
                            hb[q + c // C, c % C:c % C + 16, :] = g[c - a:c - a + 16].astype(bf16)
                assert cv.n == G and pos == 2 * E // 16

            wait(pro)
            for g in range(G):
                xs[g] = shifts(buf[0, g])
            cv = Conv(buf.at[1], 0)
            for g in range(G):
                cv.group()

            def body1(b, _):
                wait(in1(b))

                @pl.when(b + 1 < nb)
                def _():
                    start(in1(b + 1))

                @pl.when(b + 1 == nb)
                def _():
                    start(in2(0))

                blk = buf.at[pl.ds(2 + (b + 1) % 2 * U, U)]
                for u in range(U):
                    step1(blk, hc.at[pl.ds(1 + b * S, S)], b, u)
                return 0

            lax.fori_loop(0, nb, body1, 0)
            start(in2(1))

            ss = jnp.sum(acc[...].T, axis=0, keepdims=True) * (_GS * _GS)
            gx = jnp.sqrt(ss + 1e-6)
            nx = gx / (jnp.mean(gx, axis=-1, keepdims=True) + 1e-6)
            sc = (g_ref[...].astype(f32).reshape(1, E) * nx + 1.0) * _GS
            w = w2t_ref[...].astype(f32)
            w2s[...] = pltpu.bitcast((w * sc).astype(bf16), u32)
            bb = jnp.sum(w * b_ref[...].astype(f32).reshape(1, E), axis=-1, keepdims=True)
            bias[...] = jnp.broadcast_to(bb, bias.shape)

        def pass2(ys, ge):
            class XA:
                def __getitem__(self, i):
                    return jnp.concatenate([dwb[10 + i[0] * T + t, i[1], :] for t in range(T)], axis=1)
                def __setitem__(self, i, v):
                    for t in range(T):
                        dwb[10 + i[0] * T + t, i[1], :] = v[:, 128 * t:128 * t + 128]
            xa = XA()
            def xrow(blk, r, g):
                v = pltpu.bitcast(blk[r // 2, g], bf16).astype(f32)
                return v[8 * (r % 2):8 * (r % 2) + 8]

            def conv_units(blk, bi):
                for e, r in enumerate(erows):
                    rs = [jnp.broadcast_to(rsc[bi, e // 2, pl.ds((e % 2) * T + t, 1), :], (8, 128)) for t in range(T)]
                    for g in range(G):
                        cs = slice(8 * g, 8 * g + 8)
                        if e == 0:
                            a = xrow(blk, r - 1, g)
                            b = xrow(blk, r, g)
                            xa[1, cs, :] = b
                        else:
                            a = xa[e % 2, cs, :]
                            b = xa[(e + 1) % 2, cs, :]
                        n = xrow(blk, r + 1, g)
                        if e < NE - 1:
                            xa[e % 2, cs, :] = n
                        k = [dwb[t, cs, :] for t in range(9)]
                        kk = hc[bi // nb, cs, 0:128 * len(tp)].astype(f32)
                        for i, t in enumerate(tp):
                            k[t] = kk[:, 128 * i:128 * i + 128]
                        p0, p1, p2 = [], [], []
                        for t in range(T):
                            ls = slice(128 * t, 128 * t + 128)
                            at, bt, nt = a[:, ls], b[:, ls], n[:, ls]
                            p0.append(pltpu.roll(at * k[0] + bt * k[3] + nt * k[6], 1, 1))
                            p1.append(at * k[1] + bt * k[4] + nt * k[7])
                            p2.append(pltpu.roll(at * k[2] + bt * k[5] + nt * k[8], 127, 1))
                        o = []
                        for t in range(T):
                            l = jnp.where(first, p0[t - 1] if t > 0 else 0.0, p0[t])
                            rr = jnp.where(last, p2[t + 1] if t < T - 1 else 0.0, p2[t])
                            o.append((p1[t] + l + rr) * rs[t])
                        ys[e, cs, :] = jnp.concatenate(o, axis=1).astype(bf16)
                        yield

            def body2(b, _):
                wait(in2(b))
                blk = buf.at[pl.ds(2 + (b + 1) % 2 * U, U)]
                hb = hc.at[pl.ds(1 + b * S, S)]
                cu = conv_units(blk, b)

                def finish(r, gb):
                    w2v = pltpu.bitcast(w2s[...], bf16)
                    cols = []
                    for c in range(0, W, nw):
                        parts = [jnp.dot(w2v[:, k:k + ks], gb[k:k + ks, c:c + nw], preferred_element_type=f32) for k in range(0, E, ks)]
                        cols.append(sum(parts[1:], parts[0]))
                    o = jnp.concatenate(cols, axis=1)
                    o = o + jnp.concatenate([bias[...]] * T, axis=1)
                    o = o + jnp.concatenate([xrow(blk, r, g) for g in range(G)], axis=0)
                    hb[r] = o.astype(bf16)
                    return o[C - 8:, W - 128:]

                p = f = a = nu = 0
                tok = None
                for ch in pat:
                    if ch.isdigit():
                        for _ in range(int(ch)):
                            next(cu)
                            nu += 1
                    elif ch == 'P':
                        assert nu >= G * (p + 1)
                        wl = pltpu.bitcast(w1t[...], bf16)[:, :C]
                        ge[p % 2] = gelu(jnp.dot(wl, ys[p], preferred_element_type=f32)).astype(bf16)
                        p += 1
                    elif ch == 'A':
                        assert arows[a] < Q * (a + 1)
                        tok = finish(arows[a], hb[Q * a:Q * a + Q].reshape(E, W))
                        a += 1
                    elif ch == 'F':
                        assert erows[f] < Q * a and f < p <= f + 2
                        tok = finish(erows[f], ge[f % 2])
                        f += 1

                @pl.when(b + 2 < nb)
                def _():
                    start(in2(b + 2))

                @pl.when(b >= 4)
                def _():
                    wait(out2(b - 4))

                for c in out2(b):
                    c.start(priority=pri)
                return 0

            lax.fori_loop(0, nb, body2, 0)
            for b in range(nb - 4, nb):
                wait(out2(b))

        pl.run_scoped(pass1,
                      pltpu.VMEM((G, 24, W), u32),
                      pltpu.VMEM((2, C, W), f32),
                      pltpu.VMEM((8, 128), f32),
                      pltpu.VMEM((2, 8 * SS, 128), f32),
                      pltpu.VMEM((E, 128), f32),
                      pltpu.VMEM((2, G, 8, 128), u32))
        pl.run_scoped(pass2, pltpu.VMEM((NE, C, W), bf16), pltpu.VMEM((2, E, W), bf16))

    vm = pl.BlockSpec(memory_space=pltpu.VMEM)
    out = pl.pallas_call(
        kernel,
        in_specs=[pl.BlockSpec(memory_space=pl.ANY), vm, vm, vm, vm, vm],
        out_specs=pl.BlockSpec(memory_space=pl.ANY),
        out_shape=jax.ShapeDtypeStruct((H, C, W), x.dtype),
        scratch_shapes=[
            pltpu.VMEM((2 + 2 * U, G, 8, W), u32),
            pltpu.VMEM((E // 2, 128), u32),
            pltpu.VMEM((C // 2, E), u32),
            pltpu.VMEM((10 + 2 * T, C, 128), f32),
            pltpu.VMEM((nb, NE // 2, 8, 128), f32),
            pltpu.VMEM((1 + nb * S, C, W), bf16),
            pltpu.SemaphoreType.DMA((2, 2)),
            pltpu.SemaphoreType.DMA((4,)),
        ],
        compiler_params=pltpu.CompilerParams(vmem_limit_bytes=vmem, flags=flags),
    )(x5, dw, w1, w2.T, gamma, beta)
    return jnp.transpose(out.reshape(H, C, W), (0, 2, 1)).reshape(x.shape)


@jax.jit
def pallas_standalone__modern_conv_block_convnext_v2__vision_kernel(x, dw, w1, w2, grn_gamma, grn_beta):
    return build(x, dw, w1, w2, grn_gamma, grn_beta)
```

```python
import numpy as np
import jax
import jax.numpy as jnp
from jax import lax
import jax.experimental.pallas as pl
import jax.experimental.pallas.tpu as pltpu

_C1 = float(np.sqrt(2.0 / np.pi))
_C2 = _C1 * 0.044715
_S = _C2 ** (1.0 / 3.0)
_K = _C1 / _S
_GS = 0.5 / _S
f32, bf16, u32 = jnp.float32, jnp.bfloat16, jnp.uint32


def build(x, dw, w1, w2, gamma, beta, sched='12C3M12C3M8C3M8C3M8', sl=None, s0=None, se=None, pat='A6A6A6A6A6A7A7A7A7APPF7FPPF7FPPFF', vmem=128 * 2**20, flag=None, order=(1, 0), late=True, SS=9, pri=0, tp=[0, 2], nw=128, ks=384):
    U = 8
    flags = {flag: True} if flag else None
    _, H, W, C = x.shape
    E = w1.shape[1]
    T = W // 128
    G = C // 8
    P = H // 2
    nb = P // U
    R = 2 * U
    NE = 6
    erows = list(range(2, 2 + NE))
    arows = [r for r in range(R) if r not in erows]
    Q = E // C
    S = Q * (R - NE)
    x5 = jnp.transpose(x.reshape(H, W, C), (0, 2, 1)).reshape(P, 2, G, 8, W)
    import re
    parse = lambda q: [(a or 'M', int(n)) for a, n in re.findall(r'([MC]?)(\d+)', q)]
    tk = [parse((sl if u == U - 1 else s0 if u == 0 else se if 2 * u in erows else None) or sched) for u in range(U)]

    def kernel(x_hbm, dw_ref, w1_ref, w2t_ref, g_ref, b_ref, o_hbm,
               buf, w1t, w2s, dwb, rsc, hc, sin, sout):
        bias = dwb.at[9]
        xu = x_hbm.bitcast(u32)
        lane = lax.broadcasted_iota(jnp.int32, (8, 128), 1)
        sub = lax.broadcasted_iota(jnp.int32, (8, 128), 0)
        first = lane == 0
        last = lane == 127
        zero = jnp.zeros((8, 128), u32)

        def cp(src, dst, sem):
            return pltpu.make_async_copy(src, dst, sem)

        def in1(b):
            s = (b + 1) % 2
            cs = []
            for j in range(2):
                want = b * U + 2 + j
                got = jnp.minimum(want, P - U)
                cs.append(cp(xu.at[pl.ds(got, U), 1 - j],
                             buf.at[pl.ds(3 + s * U - (want - got), U), :, pl.ds(4 * j, 4)], sin.at[s, j]))
            return cs

        def in2(b):
            s = (b + 1) % 2
            return [cp(xu.at[pl.ds(b * U, U), j], buf.at[pl.ds(3 + s * U, U), :, pl.ds(4 * j, 4)], sin.at[s, j]) for j in range(2)]

        def out2(b):
            return [cp(hc.at[pl.ds(1 + b * S, R)], o_hbm.at[pl.ds(b * R, R)], sout.at[b % 4])]

        def start(cs):
            for c in cs:
                c.start()

        def wait(cs):
            for c in cs:
                c.wait()

        def gelu(z):
            return z * (1.0 + jnp.tanh(z * (_K + z * z)))

        def pass1(xs, ob, db, rsb, stt, acc, dm):
            pro = (cp(xu.at[pl.ds(0, 2), 1], buf.at[pl.ds(1, 2), :, pl.ds(0, 4)], sin.at[0, 0]),
                   cp(xu.at[pl.ds(0, 3), 0], buf.at[pl.ds(0, 3), :, pl.ds(4, 4)], sin.at[0, 1]))
            start(pro)
            start(in1(0))

            w = w1_ref[...].astype(f32)
            w = jnp.concatenate([w, jnp.zeros((128 - C, E), f32)], axis=0)
            w1t[...] = pltpu.bitcast(w.T.astype(bf16), u32)
            d = jnp.concatenate([dw_ref[i].astype(f32) for i in range(3)], axis=0)
            d = jnp.concatenate([d, jnp.zeros((9, 128 - C), f32)], axis=1)
            dt = jnp.concatenate([d, jnp.zeros((128 - 9, 128), f32)], axis=0).T
            pad_row = (lane >= 48) & (lane % 16 >= 8)
            for g in range(G):
                cols = [jnp.broadcast_to(dt[8 * g:8 * g + 8, t:t + 1], (8, 128)) for t in range(9)]
                for t in range(9):
                    dwb[t, 8 * g:8 * g + 8, :] = cols[t]
                hc[0, 8 * g:8 * g + 8, 0:128 * len(tp)] = jnp.concatenate([cols[t] for t in tp], axis=1).astype(bf16)
                halves = []
                for j in range(2):
                    m = jnp.zeros((8, 128), f32)
                    for r in range(4):
                        if 0 <= r - j < 3:
                            for s in range(3):
                                base = (r // 2) * 48 + s * 16 + (r % 2) * 8
                                m = jnp.where(lane == base + sub, cols[(r - j) * 3 + s], m)
                    halves.append(m)
                dm[0, g] = pltpu.bitcast(jnp.concatenate(halves, axis=0).astype(bf16), u32)
                halves[1] = jnp.where(pad_row, 0.0, halves[1])
                dm[1, g] = pltpu.bitcast(jnp.concatenate(halves, axis=0).astype(bf16), u32)
            acc[...] = jnp.zeros_like(acc)

            def shifts(v):
                tl = [v[:, 128 * t:128 * t + 128] for t in range(T)]
                a = [pltpu.roll(q, 1, 1) for q in tl]
                b = [pltpu.roll(q, 127, 1) for q in tl]
                l = [jnp.where(first, a[t - 1] if t > 0 else zero, a[t]) for t in range(T)]
                r = [jnp.where(last, b[t + 1] if t < T - 1 else zero, b[t]) for t in range(T)]
                return jnp.concatenate([jnp.concatenate(l, axis=1), v, jnp.concatenate(r, axis=1)], axis=0)

            def chan_mean(q, st):
                for j in range(2):
                    for t in range(T):
                        i = j * T + t
                        stt[q, SS * i:SS * i + 8, :] = st[8 * j:8 * j + 8, 128 * t:128 * t + 128]
                p = [stt[q, pl.ds(i, 8, stride=SS), :] for i in range(8)]
                return (((p[0] + p[1]) + (p[2] + p[3])) + ((p[4] + p[5]) + (p[6] + p[7]))) * (1.0 / C)

            def spread(q, j):
                return jnp.concatenate([jnp.broadcast_to(rsb[q, j * T + t:j * T + t + 1, :], (8, 128)) for t in range(T)], axis=1)

            class Conv:
                def __init__(self, s, sel, center=True):
                    self.s, self.sel, self.n, self.center = s, sel, 0, center
                    if center:
                        self.m = jnp.concatenate([spread(2, j) for j in range(2)], axis=0)

                def group(self):
                    g = self.n
                    self.n += 1
                    if self.center:
                        d = ob[g] - self.m
                        for j in range(2):
                            db[j, 8 * g:8 * g + 8, :] = d[8 * j:8 * j + 8]
                        self.s2 = d * d if g == 0 else self.s2 + d * d
                    old = xs[g]
                    new = shifts(self.s[g])
                    xs[g] = new
                    rhs = pltpu.bitcast(jnp.concatenate([old, new], axis=0), bf16)
                    lhs = pltpu.bitcast(dm[self.sel, g], bf16)[:, :96]
                    o = jnp.dot(lhs, rhs, preferred_element_type=f32)
                    ob[g] = o
                    self.s1 = o if g == 0 else self.s1 + o
                    if self.n == G:
                        if self.center:
                            rsb[0] = rsb[2]
                            rsb[1] = lax.rsqrt(chan_mean(1, self.s2) + 1e-5) * _S
                        rsb[2] = chan_mean(0, self.s1)

            def norm(j):
                return (db[j] * jnp.concatenate([spread(1, j)] * G, axis=0)).astype(bf16)

            def step1(blk, hb, bi, u):
                ys = [norm(0), norm(1)]
                if 2 * u in erows:
                    rsc[bi, erows.index(2 * u) // 2] = rsb[0:2]
                cv = Conv(blk.at[u], (bi == nb - 1).astype(jnp.int32) if u == U - 3 else 0)
                pos = 0
                for kind, n in tk[u]:
                    if kind == 'C':
                        for _ in range(n):
                            cv.group()
                        continue
                    j = order[pos // (E // 16)]
                    a = 16 * (pos % (E // 16))
                    b = a + 16 * n
                    pos += n
                    wl = pltpu.bitcast(w1t[a // 2:b // 2, :], bf16)[:, :C]
                    g = gelu(jnp.dot(wl, ys[j], preferred_element_type=f32))
                    g2 = g * g
                    sq = g2[:, 0:128]
                    for t in range(1, T):
                        sq = sq + g2[:, 128 * t:128 * t + 128]
                    acc[a:b, :] += sq
                    if 2 * u + j in arows:
                        q = Q * arows.index(2 * u + j)
                        for c in range(a, b, 16):
                            hb[q + c // C, c % C:c % C + 16, :] = g[c - a:c - a + 16].astype(bf16)
                assert cv.n == G and pos == 2 * E // 16

            wait(pro)
            buf[0, :, 0:4, :] = jnp.zeros((G, 4, W), u32)
            for g in range(G):
                xs[g] = shifts(buf[0, g])
            for k in (1, 2):
                cv = Conv(buf.at[k], 0, k == 2)
                for g in range(G):
                    cv.group()

            def body1(b, _):
                wait(in1(b))

                @pl.when(b + 1 < nb)
                def _():
                    start(in1(b + 1))

                @pl.when(b + 1 == nb)
                def _():
                    start(in2(0))

                blk = buf.at[pl.ds(3 + (b + 1) % 2 * U, U)]
                for u in range(U):
                    step1(blk, hc.at[pl.ds(1 + b * S, S)], b, u)
                return 0

            lax.fori_loop(0, nb, body1, 0)
            start(in2(1))

            ss = jnp.sum(acc[...].T, axis=0, keepdims=True) * (_GS * _GS)
            gx = jnp.sqrt(ss + 1e-6)
            nx = gx / (jnp.mean(gx, axis=-1, keepdims=True) + 1e-6)
            sc = (g_ref[...].astype(f32).reshape(1, E) * nx + 1.0) * _GS
            w = w2t_ref[...].astype(f32)
            w2s[...] = pltpu.bitcast((w * sc).astype(bf16), u32)
            bb = jnp.sum(w * b_ref[...].astype(f32).reshape(1, E), axis=-1, keepdims=True)
            bias[...] = jnp.broadcast_to(bb, bias.shape)

        def pass2(ys, ge):
            class XA:
                def __getitem__(self, i):
                    return jnp.concatenate([dwb[10 + i[0] * T + t, i[1], :] for t in range(T)], axis=1)
                def __setitem__(self, i, v):
                    for t in range(T):
                        dwb[10 + i[0] * T + t, i[1], :] = v[:, 128 * t:128 * t + 128]
            xa = XA()
            def xrow(blk, r, g):
                v = pltpu.bitcast(blk[r // 2, g], bf16).astype(f32)
                return v[8 * (r % 2):8 * (r % 2) + 8]

            def conv_units(blk, bi):
                for e, r in enumerate(erows):
                    mu, rs = [[jnp.broadcast_to(rsc[bi, e // 2, q, pl.ds((e % 2) * T + t, 1), :], (8, 128)) for t in range(T)] for q in range(2)]
                    for g in range(G):
                        cs = slice(8 * g, 8 * g + 8)
                        if e == 0:
                            a = xrow(blk, r - 1, g)
                            b = xrow(blk, r, g)
                            xa[1, cs, :] = b
                        else:
                            a = xa[e % 2, cs, :]
                            b = xa[(e + 1) % 2, cs, :]
                        n = xrow(blk, r + 1, g)
                        if e < NE - 1:
                            xa[e % 2, cs, :] = n
                        k = [dwb[t, cs, :] for t in range(9)]
                        kk = hc[bi // nb, cs, 0:128 * len(tp)].astype(f32)
                        for i, t in enumerate(tp):
                            k[t] = kk[:, 128 * i:128 * i + 128]
                        p0, p1, p2 = [], [], []
                        for t in range(T):
                            ls = slice(128 * t, 128 * t + 128)
                            at, bt, nt = a[:, ls], b[:, ls], n[:, ls]
                            p0.append(pltpu.roll(at * k[0] + bt * k[3] + nt * k[6], 1, 1))
                            p1.append(at * k[1] + bt * k[4] + nt * k[7])
                            p2.append(pltpu.roll(at * k[2] + bt * k[5] + nt * k[8], 127, 1))
                        o = []
                        for t in range(T):
                            l = jnp.where(first, p0[t - 1] if t > 0 else 0.0, p0[t])
                            rr = jnp.where(last, p2[t + 1] if t < T - 1 else 0.0, p2[t])
                            o.append((p1[t] - mu[t] + l + rr) * rs[t])
                        ys[e, cs, :] = jnp.concatenate(o, axis=1).astype(bf16)
                        yield

            def body2(b, _):
                wait(in2(b))
                blk = buf.at[pl.ds(3 + (b + 1) % 2 * U, U)]
                hb = hc.at[pl.ds(1 + b * S, S)]
                cu = conv_units(blk, b)

                def finish(r, gb):
                    w2v = pltpu.bitcast(w2s[...], bf16)
                    cols = []
                    for c in range(0, W, nw):
                        parts = [jnp.dot(w2v[:, k:k + ks], gb[k:k + ks, c:c + nw], preferred_element_type=f32) for k in range(0, E, ks)]
                        cols.append(sum(parts[1:], parts[0]))
                    o = jnp.concatenate(cols, axis=1)
                    o = o + jnp.concatenate([bias[...]] * T, axis=1)
                    o = o + jnp.concatenate([xrow(blk, r, g) for g in range(G)], axis=0)
                    hb[r] = o.astype(bf16)
                    return o[C - 8:, W - 128:]

                p = f = a = nu = 0
                tok = None
                for ch in pat:
                    if ch.isdigit():
                        for _ in range(int(ch)):
                            next(cu)
                            nu += 1
                    elif ch == 'P':
                        assert nu >= G * (p + 1)
                        wl = pltpu.bitcast(w1t[...], bf16)[:, :C]
                        ge[p % 2] = gelu(jnp.dot(wl, ys[p], preferred_element_type=f32)).astype(bf16)
                        p += 1
                    elif ch == 'A':
                        assert arows[a] < Q * (a + 1)
                        tok = finish(arows[a], hb[Q * a:Q * a + Q].reshape(E, W))
                        a += 1
                    elif ch == 'F':
                        assert erows[f] < Q * a and f < p <= f + 2
                        tok = finish(erows[f], ge[f % 2])
                        f += 1

                @pl.when(b + 2 < nb)
                def _():
                    start(in2(b + 2))

                @pl.when(b >= 4)
                def _():
                    wait(out2(b - 4))

                for c in out2(b):
                    c.start(priority=pri)
                return 0

            lax.fori_loop(0, nb, body2, 0)
            for b in range(nb - 4, nb):
                wait(out2(b))

        pl.run_scoped(pass1,
                      pltpu.VMEM((G, 24, W), u32),
                      pltpu.VMEM((G, 16, W), f32),
                      pltpu.VMEM((2, C, W), f32),
                      pltpu.VMEM((3, 8, 128), f32),
                      pltpu.VMEM((2, 8 * SS, 128), f32),
                      pltpu.VMEM((E, 128), f32),
                      pltpu.VMEM((2, G, 8, 128), u32))
        pl.run_scoped(pass2, pltpu.VMEM((NE, C, W), bf16), pltpu.VMEM((2, E, W), bf16))

    vm = pl.BlockSpec(memory_space=pltpu.VMEM)
    out = pl.pallas_call(
        kernel,
        in_specs=[pl.BlockSpec(memory_space=pl.ANY), vm, vm, vm, vm, vm],
        out_specs=pl.BlockSpec(memory_space=pl.ANY),
        out_shape=jax.ShapeDtypeStruct((H, C, W), x.dtype),
        scratch_shapes=[
            pltpu.VMEM((3 + 2 * U, G, 8, W), u32),
            pltpu.VMEM((E // 2, 128), u32),
            pltpu.VMEM((C // 2, E), u32),
            pltpu.VMEM((10 + 2 * T, C, 128), f32),
            pltpu.VMEM((nb, NE // 2, 2, 8, 128), f32),
            pltpu.VMEM((1 + nb * S, C, W), bf16),
            pltpu.SemaphoreType.DMA((2, 2)),
            pltpu.SemaphoreType.DMA((4,)),
        ],
        compiler_params=pltpu.CompilerParams(vmem_limit_bytes=vmem, flags=flags),
    )(x5, dw, w1, w2.T, gamma, beta)
    return jnp.transpose(out.reshape(H, C, W), (0, 2, 1)).reshape(x.shape)


@jax.jit
def pallas_standalone__modern_conv_block_convnext_v2__vision_kernel(x, dw, w1, w2, grn_gamma, grn_beta):
    return build(x, dw, w1, w2, grn_gamma, grn_beta)
```

```python
import numpy as np
import jax
import jax.numpy as jnp
from jax import lax
import jax.experimental.pallas as pl
import jax.experimental.pallas.tpu as pltpu

_C1 = float(np.sqrt(2.0 / np.pi))
_S = (_C1 * 0.044715) ** (1.0 / 3.0)
_K = _C1 / _S
_GS = 0.5 / _S

_U = 8
_R = 2 * _U
_REDO = tuple(range(2, 8))
_KEEP = tuple(r for r in range(_R) if r not in _REDO)
_LEAD = 3
_STRIDE = 9
_CONV_AFTER = (2, 2, 2, 4, 2, 0)
_ORDER = "A6A6A6A6A6A6A6A6A6A1P1PF7F1P1PF7FPPFF"
_PACED_TAPS = (0, 2)

f32, bf16, u32 = jnp.float32, jnp.bfloat16, jnp.uint32


def _gelu(z):
    return z * (1.0 + jnp.tanh(z * (_K + z * z)))


def _start(copies):
    for c in copies:
        c.start()


def _wait(copies):
    for c in copies:
        c.wait()


def _kernel(x_hbm, dw_ref, w1_ref, w2t_ref, gamma_ref, beta_ref, o_hbm,
            xbuf, w1t, w2s, planes, ln_cache, cache, sem_in, sem_out):
    H, C, W = o_hbm.shape
    E = w1_ref.shape[1]
    T, G, P = W // 128, C // 8, H // 2
    nb = P // _U
    Q = E // C
    S = Q * len(_KEEP)
    BIAS, XF = 9, 10

    xu = x_hbm.bitcast(u32)
    lane = lax.broadcasted_iota(jnp.int32, (8, 128), 1)
    sub = lax.broadcasted_iota(jnp.int32, (8, 128), 0)
    first = lane == 0
    last = lane == 127

    def tile(v, t):
        return v[:, 128 * t:128 * t + 128]

    def x_copy(src, parity, dst, half, n, sem):
        return pltpu.make_async_copy(
            xu.at[pl.ds(src, n), parity],
            xbuf.at[pl.ds(dst, n), :, pl.ds(4 * half, 4)], sem)

    def x_block(b):
        return xbuf.at[pl.ds(_LEAD + (b + 1) % 2 * _U, _U)]

    def cache_block(b):
        return cache.at[pl.ds(1 + b * S, S)]

    def load1(b):
        s = (b + 1) % 2
        copies = []
        for j in range(2):
            want = b * _U + _LEAD - 1 + j
            got = jnp.minimum(want, P - _U)
            copies.append(x_copy(got, 1 - j, _LEAD + s * _U - (want - got), j,
                                 _U, sem_in.at[s, j]))
        return copies

    def load2(b):
        s = (b + 1) % 2
        return [x_copy(b * _U, j, _LEAD + s * _U, j, _U, sem_in.at[s, j])
                for j in range(2)]

    def store2(b):
        return [pltpu.make_async_copy(cache.at[pl.ds(1 + b * S, _R)],
                                      o_hbm.at[pl.ds(b * _R, _R)],
                                      sem_out.at[b % 4])]

    def pass1(xs, conv, cent, stats, red, acc, band):
        head = (x_copy(0, 1, 1, 0, _LEAD - 1, sem_in.at[0, 0]),
                x_copy(0, 0, 0, 1, _LEAD, sem_in.at[0, 1]))
        _start(head)
        _start(load1(0))

        w = jnp.concatenate(
            [w1_ref[...].astype(f32), jnp.zeros((128 - C, E), f32)], axis=0)
        w1t[...] = pltpu.bitcast(w.T.astype(bf16), u32)
        d = jnp.concatenate([dw_ref[i].astype(f32) for i in range(3)], axis=0)
        d = jnp.concatenate([d, jnp.zeros((9, 128 - C), f32)], axis=1)
        dt = jnp.concatenate([d, jnp.zeros((128 - 9, 128), f32)], axis=0).T
        pad_row = (lane >= 48) & (lane % 16 >= 8)
        for g in range(G):
            cs = slice(8 * g, 8 * g + 8)
            taps = [jnp.broadcast_to(dt[cs, t:t + 1], (8, 128)) for t in range(9)]
            for t in range(9):
                planes[t, cs, :] = taps[t]
            cache[0, cs, 0:128 * len(_PACED_TAPS)] = jnp.concatenate(
                [taps[t] for t in _PACED_TAPS], axis=1).astype(bf16)
            rows = []
            for j in range(2):
                m = jnp.zeros((8, 128), f32)
                for r in range(j, j + 3):
                    for s in range(3):
                        col = (r // 2) * 48 + s * 16 + (r % 2) * 8
                        m = jnp.where(lane == col + sub, taps[(r - j) * 3 + s], m)
                rows.append(m)
            band[0, g] = pltpu.bitcast(jnp.concatenate(rows, axis=0).astype(bf16), u32)
            rows[1] = jnp.where(pad_row, 0.0, rows[1])
            band[1, g] = pltpu.bitcast(jnp.concatenate(rows, axis=0).astype(bf16), u32)
        acc[...] = jnp.zeros_like(acc)

        def shifts(v):
            zero = jnp.zeros((8, 128), u32)
            a = [pltpu.roll(tile(v, t), 1, 1) for t in range(T)]
            b = [pltpu.roll(tile(v, t), 127, 1) for t in range(T)]
            l = [jnp.where(first, a[t - 1] if t > 0 else zero, a[t]) for t in range(T)]
            r = [jnp.where(last, b[t + 1] if t < T - 1 else zero, b[t]) for t in range(T)]
            return jnp.concatenate(
                [jnp.concatenate(l, axis=1), v, jnp.concatenate(r, axis=1)], axis=0)

        def channel_mean(q, part):
            for j in range(2):
                for t in range(T):
                    i = _STRIDE * (j * T + t)
                    red[q, i:i + 8, :] = tile(part[8 * j:8 * j + 8], t)
            p = [red[q, pl.ds(i, 8, stride=_STRIDE), :] for i in range(8)]
            return (((p[0] + p[1]) + (p[2] + p[3]))
                    + ((p[4] + p[5]) + (p[6] + p[7]))) * (1.0 / C)

        def spread(q, j):
            return jnp.concatenate(
                [jnp.broadcast_to(stats[q, j * T + t:j * T + t + 1, :], (8, 128))
                 for t in range(T)], axis=1)

        def conv_groups(src, prev=None, bottom=0, center=True, keep=True):
            for g in range(G):
                if center:
                    d = conv[g] - conv[G]
                    for j in range(2):
                        cent[j, 8 * g:8 * g + 8, :] = d[8 * j:8 * j + 8]
                    s2 = d * d if g == 0 else s2 + d * d
                old = xs[g] if prev is None else jnp.concatenate(
                    [xs[g, 0:8], prev[g], xs[g, 16:24]], axis=0)
                new = shifts(src[g])
                if keep:
                    xs[g] = new
                else:
                    xs[g, 0:8] = new[0:8]
                    xs[g, 16:24] = new[16:24]
                rhs = pltpu.bitcast(jnp.concatenate([old, new], axis=0), bf16)
                lhs = pltpu.bitcast(band[bottom, g], bf16)[:, :96]
                o = jnp.dot(lhs, rhs, preferred_element_type=f32)
                conv[g] = o
                s1 = o if g == 0 else s1 + o
                if g == G - 1:
                    if center:
                        stats[0] = stats[2]
                        stats[1] = lax.rsqrt(channel_mean(1, s2) + 1e-5) * _S
                    stats[2] = channel_mean(0, s1)
                    conv[G] = jnp.concatenate([spread(2, j) for j in range(2)], axis=0)
                yield

        def pair_step(b, u):
            xb, cb = x_block(b), cache_block(b)
            y = [(cent[j] * jnp.concatenate([spread(1, j)] * G, axis=0)).astype(bf16)
                 for j in range(2)]
            if 2 * u in _REDO:
                ln_cache[b, _REDO.index(2 * u) // 2] = stats[0:2]
            groups = conv_groups(
                xb.at[u], xb.at[u - 1] if u > 0 else None,
                (b == nb - 1).astype(jnp.int32) if u == _U - _LEAD else 0,
                keep=u == _U - 1)
            slabs = [(j, e) for j in (1, 0) for e in range(0, E, 128)]
            for (j, e), n in zip(slabs, _CONV_AFTER, strict=True):
                wl = pltpu.bitcast(w1t[e // 2:e // 2 + 64, :], bf16)[:, :C]
                h = _gelu(jnp.dot(wl, y[j], preferred_element_type=f32))
                h2 = h * h
                sq = tile(h2, 0)
                for t in range(1, T):
                    sq = sq + tile(h2, t)
                acc[e:e + 128, :] += sq
                if 2 * u + j in _KEEP:
                    q = Q * _KEEP.index(2 * u + j)
                    for c in range(e, e + 128, 16):
                        cb[q + c // C, c % C:c % C + 16, :] = (
                            h[c - e:c - e + 16].astype(bf16))
                for _ in range(n):
                    next(groups)

        _wait(head)
        xbuf[0, :, 0:4, :] = jnp.zeros((G, 4, W), u32)
        for g in range(G):
            xs[g] = shifts(xbuf[0, g])
        for k in range(1, _LEAD):
            for _ in conv_groups(xbuf.at[k], center=k > 1):
                pass

        def block(b, carry):
            _wait(load1(b))

            @pl.when(b + 1 < nb)
            def _():
                _start(load1(b + 1))

            @pl.when(b + 1 == nb)
            def _():
                _start(load2(0))

            for u in range(_U):
                pair_step(b, u)
            return carry

        lax.fori_loop(0, nb, block, 0)
        _start(load2(1))

        ss = jnp.sum(acc[...].T, axis=0, keepdims=True) * (_GS * _GS)
        gx = jnp.sqrt(ss + 1e-6)
        nx = gx / (jnp.mean(gx, axis=-1, keepdims=True) + 1e-6)
        scale = (gamma_ref[...].astype(f32).reshape(1, E) * nx + 1.0) * _GS
        w = w2t_ref[...].astype(f32)
        w2s[...] = pltpu.bitcast((w * scale).astype(bf16), u32)
        shift = jnp.sum(w * beta_ref[...].astype(f32).reshape(1, E),
                        axis=-1, keepdims=True)
        planes[BIAS] = jnp.broadcast_to(shift, (C, 128))

    def pass2(ys, hs):
        def x_rows(xb, r, g):
            v = pltpu.bitcast(xb[r // 2, g], bf16).astype(f32)
            return v[8 * (r % 2):8 * (r % 2) + 8]

        def conv_units(xb, b):
            for e, r in enumerate(_REDO):
                mu, rs = [[jnp.broadcast_to(
                    ln_cache[b, e // 2, q, pl.ds((e % 2) * T + t, 1), :], (8, 128))
                    for t in range(T)] for q in range(2)]
                older, newer = XF + e % 2 * T, XF + (e + 1) % 2 * T
                for g in range(G):
                    cs = slice(8 * g, 8 * g + 8)
                    if e == 0:
                        up, mid = [[tile(x_rows(xb, q, g), t) for t in range(T)]
                                   for q in (r - 1, r)]
                        for t in range(T):
                            planes[newer + t, cs, :] = mid[t]
                    else:
                        up = [planes[older + t, cs, :] for t in range(T)]
                        mid = [planes[newer + t, cs, :] for t in range(T)]
                    down = x_rows(xb, r + 1, g)
                    if e < len(_REDO) - 1:
                        for t in range(T):
                            planes[older + t, cs, :] = tile(down, t)
                    k = [planes[t, cs, :] for t in range(9)]
                    paced = cache[b // nb, cs, 0:128 * len(_PACED_TAPS)].astype(f32)
                    for i, t in enumerate(_PACED_TAPS):
                        k[t] = tile(paced, i)
                    p0, p1, p2 = [], [], []
                    for t in range(T):
                        a, m, n = up[t], mid[t], tile(down, t)
                        p0.append(pltpu.roll(a * k[0] + m * k[3] + n * k[6], 1, 1))
                        p1.append(a * k[1] + m * k[4] + n * k[7])
                        p2.append(pltpu.roll(a * k[2] + m * k[5] + n * k[8], 127, 1))
                    o = []
                    for t in range(T):
                        left = jnp.where(first, p0[t - 1] if t > 0 else 0.0, p0[t])
                        right = jnp.where(last, p2[t + 1] if t < T - 1 else 0.0, p2[t])
                        o.append((p1[t] - mu[t] + left + right) * rs[t])
                    ys[e, cs, :] = jnp.concatenate(o, axis=1).astype(bf16)
                    yield

        def block(b, carry):
            _wait(load2(b))
            xb, cb = x_block(b), cache_block(b)
            units = conv_units(xb, b)

            def finish(r, h):
                w = pltpu.bitcast(w2s[...], bf16)
                o = jnp.concatenate(
                    [jnp.dot(w, tile(h, t), preferred_element_type=f32)
                     for t in range(T)], axis=1)
                o = o + jnp.concatenate([planes[BIAS]] * T, axis=1)
                o = o + jnp.concatenate([x_rows(xb, r, g) for g in range(G)], axis=0)
                cb[r] = o.astype(bf16)

            p = f = a = done = 0
            for op in _ORDER:
                if op == "P":
                    assert done >= G * (p + 1) and p < f + 2
                    wl = pltpu.bitcast(w1t[...], bf16)[:, :C]
                    hs[p % 2] = _gelu(
                        jnp.dot(wl, ys[p], preferred_element_type=f32)).astype(bf16)
                    p += 1
                elif op == "A":
                    assert _KEEP[a] < Q * (a + 1)
                    finish(_KEEP[a], cb[Q * a:Q * a + Q].reshape(E, W))
                    a += 1
                elif op == "F":
                    assert _REDO[f] < Q * a and f < p
                    finish(_REDO[f], hs[f % 2])
                    f += 1
                else:
                    for _ in range(int(op)):
                        next(units)
                    done += int(op)
            assert a == len(_KEEP) and f == len(_REDO)

            @pl.when(b + 2 < nb)
            def _():
                _start(load2(b + 2))

            @pl.when(b >= 4)
            def _():
                _wait(store2(b - 4))

            _start(store2(b))
            return carry

        lax.fori_loop(0, nb, block, 0)
        for b in range(nb - 4, nb):
            _wait(store2(b))

    pl.run_scoped(
        pass1,
        pltpu.VMEM((G, 24, W), u32),
        pltpu.VMEM((G + 1, 16, W), f32),
        pltpu.VMEM((2, C, W), f32),
        pltpu.VMEM((3, 8, 128), f32),
        pltpu.VMEM((2, 8 * _STRIDE, 128), f32),
        pltpu.VMEM((E, 128), f32),
        pltpu.VMEM((2, G, 8, 128), u32))
    pl.run_scoped(
        pass2,
        pltpu.VMEM((len(_REDO), C, W), bf16),
        pltpu.VMEM((2, E, W), bf16))


@jax.jit
def pallas_standalone__modern_conv_block_convnext_v2__vision_kernel(
    x: jax.Array,
    dw: jax.Array,
    w1: jax.Array,
    w2: jax.Array,
    grn_gamma: jax.Array,
    grn_beta: jax.Array,
):
    B, H, W, C = x.shape
    E = w1.shape[1]
    nb = H // _R
    assert (B, W, C, E) == (1, 512, 96, 384) and dw.shape[:2] == (3, 3)
    assert H % (2 * _R) == 0 and nb >= 4 and x.dtype == bf16

    xt = jnp.transpose(x.reshape(H, W, C), (0, 2, 1)).reshape(H // 2, 2, C // 8, 8, W)
    vmem = pl.BlockSpec(memory_space=pltpu.VMEM)
    out = pl.pallas_call(
        _kernel,
        in_specs=[pl.BlockSpec(memory_space=pl.ANY), vmem, vmem, vmem, vmem, vmem],
        out_specs=pl.BlockSpec(memory_space=pl.ANY),
        out_shape=jax.ShapeDtypeStruct((H, C, W), x.dtype),
        scratch_shapes=[
            pltpu.VMEM((_LEAD + 2 * _U, C // 8, 8, W), u32),
            pltpu.VMEM((E // 2, 128), u32),
            pltpu.VMEM((C // 2, E), u32),
            pltpu.VMEM((10 + 2 * W // 128, C, 128), f32),
            pltpu.VMEM((nb, len(_REDO) // 2, 2, 8, 128), f32),
            pltpu.VMEM((1 + nb * len(_KEEP) * E // C, C, W), bf16),
            pltpu.SemaphoreType.DMA((2, 2)),
            pltpu.SemaphoreType.DMA((4,)),
        ],
        compiler_params=pltpu.CompilerParams(vmem_limit_bytes=128 * 2**20),
    )(xt, dw, w1, w2.T, grn_gamma, grn_beta)
    return jnp.transpose(out, (0, 2, 1)).reshape(x.shape)
```

```python
import numpy as np
import jax
import jax.numpy as jnp
from jax import lax
import jax.experimental.pallas as pl
import jax.experimental.pallas.tpu as pltpu

_C1 = float(np.sqrt(2.0 / np.pi))
_S = (_C1 * 0.044715) ** (1.0 / 3.0)
_K = _C1 / _S
_GS = 0.5 / _S

_U = 8
_R = 2 * _U
_REDO = tuple(range(2, 8))
_KEEP = tuple(r for r in range(_R) if r not in _REDO)
_LEAD = 3
_STRIDE = 9
_CONV_AFTER = (2, 2, 2, 3, 3, 0)
_ORDER = "A6A6A6A6A6A6A6A6A2P1PF7F2P1PF7F2P2PFAF"
_ORDER_LAST = "A6A6A6A6A6A6A6A6A6A1PWPF7F1P2PF7FPWPFFW"
_WRITES_LAST = (((0, 2), (8, 8)), ((2, 4),), ((6, 2),))
_PACED_TAPS = (6, 8)

f32, bf16, u32 = jnp.float32, jnp.bfloat16, jnp.uint32


def _gelu(z):
    return z * (1.0 + jnp.tanh(z * (_K + z * z)))


def _start(copies):
    for c in copies:
        c.start()


def _wait(copies):
    for c in copies:
        c.wait()


def _kernel(x_hbm, dw_ref, w1_ref, w2t_ref, gamma_ref, beta_ref, o_hbm,
            xbuf, w1t, w2s, planes, ln_cache, cache, sem_in, sem_out):
    H, C, W = o_hbm.shape
    E = w1_ref.shape[1]
    T, G, P = W // 128, C // 8, H // 2
    nb = P // _U
    Q = E // C
    S = Q * len(_KEEP)
    BIAS, XF = 9, 10

    lane = lax.broadcasted_iota(jnp.int32, (8, 128), 1)
    sub = lax.broadcasted_iota(jnp.int32, (8, 128), 0)
    first = lane == 0
    last = lane == 127

    def tile(v, t):
        return v[:, 128 * t:128 * t + 128]

    def x_copy(src, parity, dst, half, n, sem):
        return pltpu.make_async_copy(
            x_hbm.at[pl.ds(src, n), parity],
            xbuf.at[pl.ds(dst, n), :, pl.ds(8 * half, 8)], sem)

    def x_block(b):
        return xbuf.at[pl.ds(_LEAD + (b + 1) % 2 * _U, _U)]

    def cache_block(b):
        return cache.at[pl.ds(1 + b * S, S)]

    def load1(b):
        s = (b + 1) % 2
        copies = []
        for j in range(2):
            want = b * _U + _LEAD - 1 + j
            got = jnp.minimum(want, P - _U)
            copies.append(x_copy(got, 1 - j, _LEAD + s * _U - (want - got), j,
                                 _U, sem_in.at[s, j]))
        return copies

    def load2(b):
        s = (b + 1) % 2
        return [x_copy(b * _U, j, _LEAD + s * _U, j, _U, sem_in.at[s, j])
                for j in range(2)]

    def store2(b):
        return [pltpu.make_async_copy(cache.at[pl.ds(1 + b * S, _R)],
                                      o_hbm.at[pl.ds(b * _R, _R)],
                                      sem_out.at[b % 4])]

    def store_rows(b, r, n):
        return pltpu.make_async_copy(cache.at[pl.ds(1 + b * S + r, n)],
                                     o_hbm.at[pl.ds(b * _R + r, n)],
                                     sem_out.at[4])

    def pass1(xs, conv, cent, stats, red, acc, band):
        head = (x_copy(0, 1, 1, 0, _LEAD - 1, sem_in.at[0, 0]),
                x_copy(0, 0, 0, 1, _LEAD, sem_in.at[0, 1]))
        _start(head)
        _start(load1(0))

        w = jnp.concatenate(
            [w1_ref[...].astype(f32), jnp.zeros((128 - C, E), f32)], axis=0)
        w1t[...] = pltpu.bitcast(w.T.astype(bf16), u32)
        d = jnp.concatenate([dw_ref[i].astype(f32) for i in range(3)], axis=0)
        d = jnp.concatenate([d, jnp.zeros((9, 128 - C), f32)], axis=1)
        dt = jnp.concatenate([d, jnp.zeros((128 - 9, 128), f32)], axis=0).T
        pad_row = (lane >= 48) & (lane % 16 >= 8)
        for g in range(G):
            cs = slice(8 * g, 8 * g + 8)
            taps = [jnp.broadcast_to(dt[cs, t:t + 1], (8, 128)) for t in range(9)]
            for t in range(9):
                planes[t, cs, :] = taps[t]
            cache[0, cs, 0:128 * len(_PACED_TAPS)] = jnp.concatenate(
                [taps[t] for t in _PACED_TAPS], axis=1).astype(bf16)
            rows = []
            for j in range(2):
                m = jnp.zeros((8, 128), f32)
                for r in range(j, j + 3):
                    for s in range(3):
                        col = (r // 2) * 48 + s * 16 + (r % 2) * 8
                        m = jnp.where(lane == col + sub, taps[(r - j) * 3 + s], m)
                rows.append(m)
            band[0, g] = pltpu.bitcast(jnp.concatenate(rows, axis=0).astype(bf16), u32)
            rows[1] = jnp.where(pad_row, 0.0, rows[1])
            band[1, g] = pltpu.bitcast(jnp.concatenate(rows, axis=0).astype(bf16), u32)
        acc[...] = jnp.zeros_like(acc)

        def shifts(v):
            v = pltpu.bitcast(v, u32)
            zero = jnp.zeros((8, 128), u32)
            a = [pltpu.roll(tile(v, t), 1, 1) for t in range(T)]
            b = [pltpu.roll(tile(v, t), 127, 1) for t in range(T)]
            l = [jnp.where(first, a[t - 1] if t > 0 else zero, a[t]) for t in range(T)]
            r = [jnp.where(last, b[t + 1] if t < T - 1 else zero, b[t]) for t in range(T)]
            return jnp.concatenate(
                [jnp.concatenate(l, axis=1), v, jnp.concatenate(r, axis=1)], axis=0)

        def channel_mean(q, part):
            for j in range(2):
                for t in range(T):
                    i = _STRIDE * (j * T + t)
                    red[q, i:i + 8, :] = tile(part[8 * j:8 * j + 8], t)
            p = [red[q, pl.ds(i, 8, stride=_STRIDE), :] for i in range(8)]
            return (((p[0] + p[1]) + (p[2] + p[3]))
                    + ((p[4] + p[5]) + (p[6] + p[7]))) * (1.0 / C)

        def spread(q, j):
            return jnp.concatenate(
                [jnp.broadcast_to(stats[q, j * T + t:j * T + t + 1, :], (8, 128))
                 for t in range(T)], axis=1)

        def conv_groups(src, bottom=0, center=True):
            for g in range(G):
                if center:
                    d = conv[g] - conv[G]
                    for j in range(2):
                        cent[j, 8 * g:8 * g + 8, :] = d[8 * j:8 * j + 8]
                    s2 = d * d if g == 0 else s2 + d * d
                old = xs[g]
                new = shifts(src[g])
                xs[g] = new
                rhs = pltpu.bitcast(jnp.concatenate([old, new], axis=0), bf16)
                lhs = pltpu.bitcast(band[bottom, g], bf16)[:, :96]
                o = jnp.dot(lhs, rhs, preferred_element_type=f32)
                conv[g] = o
                s1 = o if g == 0 else s1 + o
                if g == G - 1:
                    if center:
                        stats[0] = stats[2]
                        stats[1] = lax.rsqrt(channel_mean(1, s2) + 1e-5) * _S
                    stats[2] = channel_mean(0, s1)
                    conv[G] = jnp.concatenate([spread(2, j) for j in range(2)], axis=0)
                yield

        def pair_step(b, u):
            xb, cb = x_block(b), cache_block(b)
            y = [(cent[j] * jnp.concatenate([spread(1, j)] * G, axis=0)).astype(bf16)
                 for j in range(2)]
            if 2 * u in _REDO:
                ln_cache[b, _REDO.index(2 * u) // 2] = stats[0:2]
            groups = conv_groups(
                xb.at[u], (b == nb - 1).astype(jnp.int32) if u == _U - _LEAD else 0)
            slabs = [(j, e) for e in range(0, E, 128) for j in (1, 0)]
            for (j, e), n in zip(slabs, _CONV_AFTER, strict=True):
                wl = pltpu.bitcast(w1t[e // 2:e // 2 + 64, :], bf16)[:, :C]
                h = _gelu(jnp.dot(wl, y[j], preferred_element_type=f32))
                h2 = h * h
                sq = tile(h2, 0)
                for t in range(1, T):
                    sq = sq + tile(h2, t)
                acc[e:e + 128, :] += sq
                if 2 * u + j in _KEEP:
                    q = Q * _KEEP.index(2 * u + j)
                    for c in range(e, e + 128, 16):
                        cb[q + c // C, c % C:c % C + 16, :] = (
                            h[c - e:c - e + 16].astype(bf16))
                for _ in range(n):
                    next(groups)

        _wait(head)
        xbuf[0, :, 0:8, :] = jnp.zeros((G, 8, W), bf16)
        for g in range(G):
            xs[g] = shifts(xbuf[0, g])
        for k in range(1, _LEAD):
            for _ in conv_groups(xbuf.at[k], center=k > 1):
                pass

        def block(b, carry):
            _wait(load1(b))

            @pl.when(b + 1 < nb)
            def _():
                _start(load1(b + 1))

            @pl.when(b + 1 == nb)
            def _():
                _start(load2(0))

            for u in range(_U):
                pair_step(b, u)
            return carry

        lax.fori_loop(0, nb, block, 0)
        _start(load2(1))

        ss = jnp.sum(acc[...].T, axis=0, keepdims=True) * (_GS * _GS)
        gx = jnp.sqrt(ss + 1e-6)
        nx = gx / (jnp.mean(gx, axis=-1, keepdims=True) + 1e-6)
        scale = (gamma_ref[...].astype(f32).reshape(1, E) * nx + 1.0) * _GS
        w = w2t_ref[...].astype(f32)
        w2s[...] = pltpu.bitcast((w * scale).astype(bf16), u32)
        shift = jnp.sum(w * beta_ref[...].astype(f32).reshape(1, E),
                        axis=-1, keepdims=True)
        planes[BIAS] = jnp.broadcast_to(shift, (C, 128))

    def pass2(ys, hs):
        def x_rows(xb, r, g):
            return xb[r // 2, g, 8 * (r % 2):8 * (r % 2) + 8, :].astype(f32)

        def conv_units(xb, b):
            for e, r in enumerate(_REDO):
                mu, rs = [[jnp.broadcast_to(
                    ln_cache[b, e // 2, q, pl.ds((e % 2) * T + t, 1), :], (8, 128))
                    for t in range(T)] for q in range(2)]
                older, newer = XF + e % 2 * T, XF + (e + 1) % 2 * T
                for g in range(G):
                    cs = slice(8 * g, 8 * g + 8)
                    if e == 0:
                        up, mid = [[tile(x_rows(xb, q, g), t) for t in range(T)]
                                   for q in (r - 1, r)]
                        for t in range(T):
                            planes[newer + t, cs, :] = mid[t]
                    else:
                        up = [planes[older + t, cs, :] for t in range(T)]
                        mid = [planes[newer + t, cs, :] for t in range(T)]
                    down = x_rows(xb, r + 1, g)
                    if e < len(_REDO) - 1:
                        for t in range(T):
                            planes[older + t, cs, :] = tile(down, t)
                    k = [planes[t, cs, :] for t in range(9)]
                    paced = cache[b // nb, cs, 0:128 * len(_PACED_TAPS)].astype(f32)
                    for i, t in enumerate(_PACED_TAPS):
                        k[t] = tile(paced, i)
                    p0, p1, p2 = [], [], []
                    for t in range(T):
                        a, m, n = up[t], mid[t], tile(down, t)
                        p0.append(pltpu.roll(a * k[0] + m * k[3] + n * k[6], 1, 1))
                        p1.append(a * k[1] + m * k[4] + n * k[7])
                        p2.append(pltpu.roll(a * k[2] + m * k[5] + n * k[8], 127, 1))
                    o = []
                    for t in range(T):
                        left = jnp.where(first, p0[t - 1] if t > 0 else 0.0, p0[t])
                        right = jnp.where(last, p2[t + 1] if t < T - 1 else 0.0, p2[t])
                        o.append((p1[t] - mu[t] + left + right) * rs[t])
                    ys[e, cs, :] = jnp.concatenate(o, axis=1).astype(bf16)
                    yield

        def compute(b, order):
            _wait(load2(b))
            xb, cb = x_block(b), cache_block(b)
            units = conv_units(xb, b)

            def finish(r, h):
                w = pltpu.bitcast(w2s[...], bf16)
                o = jnp.concatenate(
                    [jnp.dot(w, tile(h, t), preferred_element_type=f32)
                     for t in range(T)], axis=1)
                o = o + jnp.concatenate([planes[BIAS]] * T, axis=1)
                o = o + jnp.concatenate([x_rows(xb, r, g) for g in range(G)], axis=0)
                cb[r] = o.astype(bf16)

            p = f = a = done = 0
            writes = iter(_WRITES_LAST)
            for op in order:
                if op == "P":
                    assert done >= G * (p + 1) and p < f + 2
                    wl = pltpu.bitcast(w1t[...], bf16)[:, :C]
                    hs[p % 2] = _gelu(
                        jnp.dot(wl, ys[p], preferred_element_type=f32)).astype(bf16)
                    p += 1
                elif op == "A":
                    assert _KEEP[a] < Q * (a + 1)
                    finish(_KEEP[a], cb[Q * a:Q * a + Q].reshape(E, W))
                    a += 1
                elif op == "F":
                    assert _REDO[f] < Q * a and f < p
                    finish(_REDO[f], hs[f % 2])
                    f += 1
                elif op == "W":
                    for r, n in next(writes):
                        assert set(range(r, r + n)) <= set(_KEEP[:a] + _REDO[:f])
                        store_rows(b, r, n).start()
                else:
                    for _ in range(int(op)):
                        next(units)
                    done += int(op)
            assert a == len(_KEEP) and f == len(_REDO)

        def block(b):
            compute(b, _ORDER)

            @pl.when(b + 2 < nb)
            def _():
                _start(load2(b + 2))

            @pl.when(b >= 4)
            def _():
                _wait(store2(b - 4))

            _start(store2(b))
            return b + 1

        end = lax.fori_loop(0, nb - 1, lambda b, _: block(b), 0)
        compute(end, _ORDER_LAST)
        for b in range(max(nb - 5, 0), nb - 1):
            _wait(store2(b))
        _wait([store_rows(nb - 1, r, n) for w in _WRITES_LAST for r, n in w])

    pl.run_scoped(
        pass1,
        pltpu.VMEM((G, 24, W), u32),
        pltpu.VMEM((G + 1, 16, W), f32),
        pltpu.VMEM((2, C, W), f32),
        pltpu.VMEM((3, 8, 128), f32),
        pltpu.VMEM((2, 8 * _STRIDE, 128), f32),
        pltpu.VMEM((E, 128), f32),
        pltpu.VMEM((2, G, 8, 128), u32))
    pl.run_scoped(
        pass2,
        pltpu.VMEM((len(_REDO), C, W), bf16),
        pltpu.VMEM((2, E, W), bf16))


@jax.jit
def pallas_standalone__modern_conv_block_convnext_v2__vision_kernel(
    x: jax.Array,
    dw: jax.Array,
    w1: jax.Array,
    w2: jax.Array,
    grn_gamma: jax.Array,
    grn_beta: jax.Array,
):
    B, H, W, C = x.shape
    E = w1.shape[1]
    nb = H // _R
    assert (B, W, C, E) == (1, 512, 96, 384) and dw.shape[:2] == (3, 3)
    assert H % (2 * _R) == 0 and nb >= 4 and x.dtype == bf16

    xt = jnp.transpose(x.reshape(H, W, C), (0, 2, 1)).reshape(H // 2, 2, C // 8, 8, W)
    vmem = pl.BlockSpec(memory_space=pltpu.VMEM)
    out = pl.pallas_call(
        _kernel,
        in_specs=[pl.BlockSpec(memory_space=pl.ANY), vmem, vmem, vmem, vmem, vmem],
        out_specs=pl.BlockSpec(memory_space=pl.ANY),
        out_shape=jax.ShapeDtypeStruct((H, C, W), x.dtype),
        scratch_shapes=[
            pltpu.VMEM((_LEAD + 2 * _U, C // 8, 16, W), bf16),
            pltpu.VMEM((E // 2, 128), u32),
            pltpu.VMEM((C // 2, E), u32),
            pltpu.VMEM((10 + 2 * W // 128, C, 128), f32),
            pltpu.VMEM((nb, len(_REDO) // 2, 2, 8, 128), f32),
            pltpu.VMEM((1 + nb * len(_KEEP) * E // C, C, W), bf16),
            pltpu.SemaphoreType.DMA((2, 2)),
            pltpu.SemaphoreType.DMA((5,)),
        ],
        compiler_params=pltpu.CompilerParams(vmem_limit_bytes=128 * 2**20),
    )(xt, dw, w1, w2.T, grn_gamma, grn_beta)
    return jnp.transpose(out, (0, 2, 1)).reshape(x.shape)
```
